```python
import os as _os
_os.environ.setdefault("JAX_PLATFORMS", "cpu")
import jax
import jax.numpy as jnp

def _softmax(x, axis=-1):
    return jax.nn.softmax(x, axis=axis)
def _gelu(x):
    return jax.nn.gelu(x, approximate=True)
def _silu(x):
    return jax.nn.silu(x)
def _sigmoid(x):
    return jax.nn.sigmoid(x)
def _layernorm(x, axis=-1, eps=1e-5):
    m = jnp.mean(x, axis=axis, keepdims=True)
    v = jnp.var(x, axis=axis, keepdims=True)
    return (x - m) / jnp.sqrt(v + eps)
def _scatter_add(tgt, idx, src, axis=0):
    return tgt.at[idx].add(src)
def _segment_sum(src, seg, n):
    return jax.ops.segment_sum(src, seg, n)
class _Rng:
    def __init__(self, key):
        self._k = key
    def _next(self):
        self._k, sub = jax.random.split(self._k)
        return sub
    def normal(self, shape):
        return jax.random.normal(self._next(), shape, dtype=jnp.bfloat16)
    def randint(self, lo, hi, shape):
        return jax.random.randint(self._next(), shape, lo, hi, dtype=jnp.int32)
    def uniform(self, shape, lo=0.0, hi=1.0):
        return jax.random.uniform(self._next(), shape, jnp.bfloat16, lo, hi)
    def permutation(self, n):
        return jax.random.permutation(self._next(), n)


kernel_name = 'parallel_sum__sliding_block__moe_arch_mod__prompt'

def setup_inputs():
    _rng = _Rng(jax.random.key(int.from_bytes(__import__("os").urandom(4), "little")))
    _w = (lambda a: (lambda t: t.astype(jnp.bfloat16) if jnp.issubdtype(t.dtype, jnp.floating) else t)(jnp.asarray(a)))
    def _A_setup():
        B, S, D = 1, 2048, 512
        return {
            "x": _w((lambda *s: _rng.normal(s) * 0.05)(B, S, D)),
            "wqkv": _w((lambda *s: _rng.normal(s) * 0.05)(D, 3 * D)),
            "wo": _w((lambda *s: _rng.normal(s) * 0.05)(D, D)),
        }
    _A_in = _A_setup()

    def _B_setup():
        B, S, D, F, C = 1, 2048, 512, 1376, 1
        return {
            "x": _w((lambda *s: _rng.normal(s) * 0.05)(B, S, D)),
            "w_r": _w((lambda *s: _rng.normal(s) * 0.05)(D)),
            "w_gate": _w((lambda *s: _rng.normal(s) * 0.05)(D, F)),
            "w_up": _w((lambda *s: _rng.normal(s) * 0.05)(D, F)),
            "w_down": _w((lambda *s: _rng.normal(s) * 0.05)(F, D)),
        }
    _B_in = _B_setup()

    return {
        "A_x": _A_in["x"],
        "A_wqkv": _A_in["wqkv"],
        "A_wo": _A_in["wo"],
        "B_x": _B_in["x"],
        "B_w_r": _B_in["w_r"],
        "B_w_gate": _B_in["w_gate"],
        "B_w_up": _B_in["w_up"],
        "B_w_down": _B_in["w_down"],
    }

def reference(A_x, A_wqkv, A_wo, B_x, B_w_r, B_w_gate, B_w_up, B_w_down):
    def _A_ref(x, wqkv, wo):
        B, S, D = x.shape
        H = 32; Dh = D // H; W = 256
        qkv = (lambda x, *d: x.transpose(*d))((x @ wqkv).reshape(B, S, 3, H, Dh), 2, 0, 3, 1, 4)
        q, k, v = qkv[0], qkv[1], qkv[2]
        scores = jnp.einsum("bhqd,bhkd->bhqk", q, k) * (Dh ** -0.5)
        idx = jnp.arange(S)
        mask = (idx[:, None] - idx[None, :] >= 0) & (idx[:, None] - idx[None, :] < W)
        scores = jnp.where(mask[None, None], scores, -1e9)
        p = _softmax(scores, axis=-1)
        o = jnp.einsum("bhqk,bhkd->bhqd", p, v)
        return (lambda x, *d: x.transpose(*d))(o, 0, 2, 1, 3).reshape(B, S, D) @ wo

    def _B_ref(x, w_r, w_gate, w_up, w_down):
        B, S, D = x.shape
        C = 1
        r = x @ w_r
        idx = jnp.argsort(-r, axis=-1)[:, :C]
        idx_e = jnp.repeat(idx.reshape(B, C, 1), D, axis=2)
        x_sel = jnp.take_along_axis(x, idx_e, axis=1)
        g = _silu(x_sel @ w_gate)
        u = x_sel @ w_up
        y = (g * u) @ w_down
        r_sel = _sigmoid(jnp.take_along_axis(r, idx, axis=1))
        y = y * r_sel.reshape(B, C, 1)
        b_off = (jnp.arange(B) * S).reshape(B, 1)
        flat_idx = (idx + b_off).reshape(B * C)
        zero = (x * 0.0).reshape(B * S, D)
        upd = _scatter_add(zero, flat_idx, y.reshape(B * C, D), axis=0)
        return x + upd.reshape(B, S, D)

    x = A_x
    xn = _layernorm(x, axis=-1)
    return x + _A_ref(xn, A_wqkv, A_wo) + _B_ref(xn, B_w_r, B_w_gate, B_w_up, B_w_down)
```

```python
import jax
import jax.numpy as jnp
from jax import lax
import jax.experimental.pallas as pl
import jax.experimental.pallas.tpu as pltpu

S, D, H, DH, W, F = 2048, 512, 32, 16, 256, 1376
BQ = 128
NB = S // BQ
KW = 3 * BQ
HG = 128 // DH
CH = 256
NCH = S // CH
HQ = 4
NQ = H // HQ
EPI_AT = 1
EPS = 1e-5
NEG = -1e9
QSCALE = DH ** -0.5 * 1.4426950408889634
BF = jnp.bfloat16
F32 = jnp.float32
NT = (((1,), (1,)), ((), ()))

_SEM_X = 0
_SEM_WQKV, _SEM_WO, _SEM_WR, _SEM_WG, _SEM_WU, _SEM_WD = range(NCH, NCH + 6)
_NSEM = NCH + 6


def _kernel(x_hbm, wqkv_hbm, wo_hbm, wr_hbm, wgT_hbm, wuT_hbm, wd_hbm, o_ref,
            x_scr, wqkv_scr, wo_scr, wr_scr, wgT_scr, wuT_scr, wd_scr,
            xn_scr, qT_scr, k_scr, vT_scr, r_scr, y_scr, idx_scr, wT_scr, woT_scr,
            s_scr, oT_scr, sems):
    i = pl.program_id(0)

    def x_copy(c):
        rows = pl.ds(pl.multiple_of(c * CH, CH), CH)
        return pltpu.make_async_copy(x_hbm.at[rows], x_scr.at[rows], sems.at[_SEM_X + c])

    def w_copies():
        return [
            pltpu.make_async_copy(wqkv_hbm, wqkv_scr, sems.at[_SEM_WQKV]),
            pltpu.make_async_copy(wr_hbm, wr_scr, sems.at[_SEM_WR]),
            pltpu.make_async_copy(wo_hbm, wo_scr, sems.at[_SEM_WO]),
            pltpu.make_async_copy(wgT_hbm, wgT_scr, sems.at[_SEM_WG]),
            pltpu.make_async_copy(wuT_hbm, wuT_scr, sems.at[_SEM_WU]),
            pltpu.make_async_copy(wd_hbm, wd_scr, sems.at[_SEM_WD]),
        ]

    def prologue():
        c_wqkv, c_wr, c_wo, c_wg, c_wu, c_wd = w_copies()
        x_copy(0).start()
        c_wqkv.start()
        c_wr.start()
        for c in range(1, NCH):
            x_copy(c).start()
        c_wo.start()
        c_wg.start()
        c_wu.start()
        c_wd.start()

        k_scr[0:BQ, :] = jnp.zeros((BQ, D), BF)
        vT_scr[:, 0:BQ] = jnp.zeros((D, BQ), BF)

        c_wqkv.wait()
        c_wr.wait()
        wT_scr[0:D, :] = wqkv_scr[:, 0:D].T
        wT_scr[D:2 * D, :] = wqkv_scr[:, 2 * D:3 * D].T

        def layernorm(c):
            r0 = pl.multiple_of(c * CH, CH)
            x_copy(c).wait()
            xf = x_scr[pl.ds(r0, CH), :].astype(F32)
            mu = jnp.mean(xf, axis=-1, keepdims=True)
            xc = xf - mu
            var = jnp.mean(xc * xc, axis=-1, keepdims=True)
            xn = (xc * lax.rsqrt(var + EPS)).astype(BF)
            xn_scr[pl.ds(r0, CH), :] = xn
            r = jnp.sum(xn.astype(F32) * wr_scr[...].astype(F32), axis=-1, keepdims=True)
            r_scr[pl.ds(r0, CH), :] = r.astype(BF).astype(F32)

        def project(c):
            r0 = pl.multiple_of(c * CH, CH)
            xn = xn_scr[pl.ds(r0, CH), :]
            k = jnp.dot(xn, wqkv_scr[:, D:2 * D], preferred_element_type=F32)
            k_scr[pl.ds(r0 + BQ, CH), :] = k.astype(BF)
            qvT = lax.dot_general(wT_scr[...], xn, NT, preferred_element_type=F32)
            qT_scr[:, pl.ds(r0, CH)] = (qvT[0:D, :] * QSCALE).astype(BF)
            vT_scr[:, pl.ds(r0 + BQ, CH)] = qvT[D:2 * D, :].astype(BF)

        layernorm(0)

        def chunk(c, carry):
            project(c)
            layernorm(c + 1)
            return carry

        lax.fori_loop(0, NCH - 1, chunk, 0)
        project(NCH - 1)

        c_wo.wait()
        woT_scr[...] = wo_scr[...].T

        r_all = r_scr[...]
        rmax = jnp.max(r_all)
        rows = lax.broadcasted_iota(jnp.int32, (S, 1), 0)
        idx = jnp.min(jnp.where(r_all == rmax, rows, S))
        idx_scr[0] = idx

        base = pl.multiple_of((idx // 16) * 16, 16)
        tile = xn_scr[pl.ds(base, 16), :].astype(F32)
        trow = lax.broadcasted_iota(jnp.int32, (16, D), 0)
        xsel = jnp.sum(jnp.where(trow == idx - base, tile, 0.0), axis=0, keepdims=True)
        xsel = jnp.broadcast_to(xsel, (16, D)).astype(BF)
        c_wg.wait()
        c_wu.wait()
        c_wd.wait()
        g = lax.dot_general(xsel, wgT_scr[...], NT, preferred_element_type=F32)
        u = lax.dot_general(xsel, wuT_scr[...], NT, preferred_element_type=F32)
        g = g.astype(BF).astype(F32)
        u = u.astype(BF).astype(F32)
        hmid = (g * jax.nn.sigmoid(g)) * u
        y = jnp.dot(hmid.astype(BF), wd_scr[...], preferred_element_type=F32)
        y_scr[...] = y[0:8, :] * jax.nn.sigmoid(rmax)

    zero16 = jnp.zeros((DH, BQ), BF)

    def key_base(blk, nt):
        return pl.multiple_of((blk + 2 - nt) * BQ, BQ)

    def qk(blk, j, nt):
        nk = nt * BQ
        q0 = pl.multiple_of(blk * BQ, BQ)
        g, part = divmod(j * HQ, HG)
        kg = k_scr[pl.ds(key_base(blk, nt), nk), g * 128:(g + 1) * 128]
        qTg = qT_scr[g * 128:(g + 1) * 128, pl.ds(q0, BQ)]
        cols = []
        for b in range(HQ):
            hh = part + b
            cols.append(jnp.concatenate(
                [qTg[r * DH:(r + 1) * DH, :] if r == hh else zero16 for r in range(HG)],
                axis=0))
        qm = jnp.concatenate(cols, axis=1)
        s_scr[j % 2, 0:nk, :] = jnp.dot(kg, qm, preferred_element_type=F32)

    def attention(blk, first):
        nt = 1 if first else 3
        nk = nt * BQ
        k0 = key_base(blk, nt)
        krow = lax.broadcasted_iota(jnp.int32, (BQ, BQ), 0)
        qcol = lax.broadcasted_iota(jnp.int32, (BQ, BQ), 1)
        diag_ok = jnp.concatenate([krow <= qcol] * HQ, axis=1)
        if not first:
            far = jnp.where(blk >= 2, 0, 2 * BQ)
            far_ok = jnp.concatenate([krow - qcol > far] * HQ, axis=1)

        oT = []

        def softmax_pv(j):
            if first:
                sT = jnp.where(diag_ok, s_scr[j % 2, 0:BQ, :], NEG)
            else:
                sT = jnp.concatenate([
                    jnp.where(far_ok, s_scr[j % 2, 0:BQ, :], NEG),
                    s_scr[j % 2, BQ:2 * BQ, :],
                    jnp.where(diag_ok, s_scr[j % 2, 2 * BQ:3 * BQ, :], NEG)], axis=0)
            m = jnp.max(sT, axis=0, keepdims=True)
            p = jnp.exp2(sT - m)
            l = jnp.sum(p, axis=0, keepdims=True)
            for b in range(HQ):
                h = j * HQ + b
                vTh = vT_scr[h * DH:(h + 1) * DH, pl.ds(k0, nk)]
                oh = lax.dot_general(vTh, p[:, b * BQ:(b + 1) * BQ], (((1,), (0,)), ((), ())),
                                     preferred_element_type=F32)
                oT.append((oh / l[:, b * BQ:(b + 1) * BQ]).astype(BF))

        if first:
            qk(blk, 0, nt)
        for j in range(NQ):
            if j + 1 < NQ:
                qk(blk, j + 1, nt)
            else:
                qk(jnp.minimum(blk + 1, NB - 1), 0, 3)
            if not first and j == EPI_AT:
                epilogue(blk - 1)
            softmax_pv(j)
        oT_scr[blk % 2] = jnp.concatenate(oT, axis=0)

    def epilogue(blk):
        q0 = pl.multiple_of(blk * BQ, BQ)
        aT = jnp.dot(woT_scr[...], oT_scr[blk % 2], preferred_element_type=F32)
        a = aT.T
        xf = x_scr[pl.ds(q0, BQ), :].astype(F32)
        xn = xn_scr[pl.ds(q0, BQ), :].astype(F32)
        grow = lax.broadcasted_iota(jnp.int32, (BQ, D), 0) + q0
        upd = xn * 0.0 + jnp.where(grow == idx_scr[0], y_scr[0:1, :], 0.0)
        o_ref[...] = (xf + a + (xn + upd)).astype(o_ref.dtype)

    @pl.when(i == 0)
    def _():
        prologue()
        attention(i, True)

    @pl.when(jnp.logical_and(i >= 1, i < NB))
    def _():
        attention(i, False)

    @pl.when(i == NB)
    def _():
        epilogue(i - 1)


@jax.jit
def pallas_parallel_sum__sliding_block__moe_arch_mod__prompt_kernel(
    A_x, A_wqkv, A_wo, B_x, B_w_r, B_w_gate, B_w_up, B_w_down):
    del B_x
    x = A_x.reshape(S, D)
    wr = B_w_r.reshape(1, D)
    hbm = pl.BlockSpec(memory_space=pl.ANY)
    vm = pltpu.VMEM
    out = pl.pallas_call(
        _kernel,
        grid=(NB + 1,),
        in_specs=[hbm] * 7,
        out_specs=pl.BlockSpec((BQ, D), lambda i: (jnp.maximum(i - 1, 0), 0)),
        out_shape=jax.ShapeDtypeStruct((S, D), A_x.dtype),
        scratch_shapes=[
            vm((S, D), BF), vm((D, 3 * D), BF), vm((D, D), BF), vm((1, D), BF),
            vm((F, D), BF), vm((F, D), BF), vm((F, D), BF),
            vm((S, D), BF),
            vm((D, S), BF),
            vm((S + BQ, D), BF),
            vm((D, S + BQ), BF),
            vm((S, 1), F32),
            vm((8, D), F32),
            pltpu.SMEM((1,), jnp.int32),
            vm((2 * D, D), BF), vm((D, D), BF),
            vm((2, KW, HQ * BQ), F32),
            vm((2, D, BQ), BF),
            pltpu.SemaphoreType.DMA((_NSEM,)),
        ],
        compiler_params=pltpu.CompilerParams(
            dimension_semantics=("arbitrary",), vmem_limit_bytes=100 * 1024 * 1024),
    )(x, A_wqkv, A_wo, wr, B_w_gate.T, B_w_up.T, B_w_down)
    return out.reshape(A_x.shape)
```

```python
import jax
import jax.numpy as jnp
from jax import lax
import jax.experimental.pallas as pl
import jax.experimental.pallas.tpu as pltpu

S, D, H, DH, W, F = 2048, 512, 32, 16, 256, 1376
BQ = 128
NB = S // BQ
KW = 3 * BQ
HG = 128 // DH
CH = 256
NCH = S // CH
HQ = 4
NQ = H // HQ
EPI_AT = 1
EPS = 1e-5
LOG2E = 1.4426950408889634
QSCALE = DH ** -0.5 * LOG2E
NEG = -1e9 * LOG2E
BF = jnp.bfloat16
F32 = jnp.float32
NT = (((1,), (1,)), ((), ()))

_SEM_X = 0
_SEM_WQKV, _SEM_WO, _SEM_WR, _SEM_WG, _SEM_WU, _SEM_WD = range(NCH, NCH + 6)
_NSEM = NCH + 6


def _kernel(x_hbm, wqkv_hbm, wo_hbm, wr_hbm, wgT_hbm, wuT_hbm, wd_hbm, o_hbm,
            x_scr, wqkv_scr, wo_scr, wr_scr, wgT_scr, wuT_scr, wd_scr,
            xn_scr, qT_scr, k_scr, vT_scr, r_scr, y_scr, idx_scr, wT_scr, woT_scr,
            s_scr, oT_scr, o_buf, sems, osems):

    def x_copy(c):
        rows = pl.ds(pl.multiple_of(c * CH, CH), CH)
        return pltpu.make_async_copy(x_hbm.at[rows], x_scr.at[rows], sems.at[_SEM_X + c])

    def w_copies():
        return [
            pltpu.make_async_copy(wqkv_hbm, wqkv_scr, sems.at[_SEM_WQKV]),
            pltpu.make_async_copy(wr_hbm, wr_scr, sems.at[_SEM_WR]),
            pltpu.make_async_copy(wo_hbm, wo_scr, sems.at[_SEM_WO]),
            pltpu.make_async_copy(wgT_hbm, wgT_scr, sems.at[_SEM_WG]),
            pltpu.make_async_copy(wuT_hbm, wuT_scr, sems.at[_SEM_WU]),
            pltpu.make_async_copy(wd_hbm, wd_scr, sems.at[_SEM_WD]),
        ]

    def prologue():
        c_wqkv, c_wr, c_wo, c_wg, c_wu, c_wd = w_copies()
        x_copy(0).start()
        c_wqkv.start()
        c_wr.start()
        for c in range(1, NCH):
            x_copy(c).start()
        c_wo.start()
        c_wg.start()
        c_wu.start()
        c_wd.start()

        k_scr[0:BQ, :] = jnp.zeros((BQ, D), BF)
        vT_scr[:, 0:BQ] = jnp.zeros((D, BQ), BF)

        def layernorm(c):
            r0 = pl.multiple_of(c * CH, CH)
            x_copy(c).wait()
            xf = x_scr[pl.ds(r0, CH), :].astype(F32)
            mu = jnp.mean(xf, axis=-1, keepdims=True)
            xc = xf - mu
            var = jnp.mean(xc * xc, axis=-1, keepdims=True)
            xn = (xc * lax.rsqrt(var + EPS)).astype(BF)
            xn_scr[pl.ds(r0, CH), :] = xn
            r = jnp.sum(xn.astype(F32) * wr_scr[...].astype(F32), axis=-1, keepdims=True)
            r_scr[pl.ds(r0, CH), :] = r.astype(BF).astype(F32)
            return xn

        def project(c, xn):
            r0 = pl.multiple_of(c * CH, CH)
            k = jnp.dot(xn, wqkv_scr[:, D:2 * D], preferred_element_type=F32)
            k_scr[pl.ds(r0 + BQ, CH), :] = k.astype(BF)
            qvT = lax.dot_general(wT_scr[...], xn, NT, preferred_element_type=F32)
            qT_scr[:, pl.ds(r0, CH)] = (qvT[0:D, :] * QSCALE).astype(BF)
            vT_scr[:, pl.ds(r0 + BQ, CH)] = qvT[D:2 * D, :].astype(BF)

        def chunk(c, xn):
            xn_next = layernorm(c + 1)
            project(c, xn)
            return xn_next

        c_wr.wait()
        xn0 = layernorm(0)
        c_wqkv.wait()
        wT_scr[0:D, :] = wqkv_scr[:, 0:D].T
        wT_scr[D:2 * D, :] = wqkv_scr[:, 2 * D:3 * D].T
        xn_last = lax.fori_loop(0, NCH - 1, chunk, xn0)
        c_wo.wait()
        c_wg.wait()
        c_wu.wait()
        c_wd.wait()
        project(NCH - 1, xn_last)

        woT_scr[...] = wo_scr[...].T

        r_all = r_scr[...]
        rmax = jnp.max(r_all)
        rows = lax.broadcasted_iota(jnp.int32, (S, 1), 0)
        idx = jnp.min(jnp.where(r_all == rmax, rows, S))
        idx_scr[0] = idx

        base = pl.multiple_of((idx // 16) * 16, 16)
        tile = xn_scr[pl.ds(base, 16), :].astype(F32)
        trow = lax.broadcasted_iota(jnp.int32, (16, D), 0)
        xsel = jnp.sum(jnp.where(trow == idx - base, tile, 0.0), axis=0, keepdims=True)
        xsel = jnp.broadcast_to(xsel, (16, D)).astype(BF)
        g = lax.dot_general(xsel, wgT_scr[...], NT, preferred_element_type=F32)
        u = lax.dot_general(xsel, wuT_scr[...], NT, preferred_element_type=F32)
        g = g.astype(BF).astype(F32)
        u = u.astype(BF).astype(F32)
        hmid = (g * jax.nn.sigmoid(g)) * u
        y = jnp.dot(hmid.astype(BF), wd_scr[...], preferred_element_type=F32)
        y_scr[...] = y[0:8, :] * jax.nn.sigmoid(rmax)

    zero16 = jnp.zeros((DH, BQ), BF)

    def key_base(blk, nt):
        return pl.multiple_of((blk + 2 - nt) * BQ, BQ)

    def qk(blk, j, nt):
        nk = nt * BQ
        q0 = pl.multiple_of(blk * BQ, BQ)
        g, part = divmod(j * HQ, HG)
        kg = k_scr[pl.ds(key_base(blk, nt), nk), g * 128:(g + 1) * 128]
        qTg = qT_scr[g * 128:(g + 1) * 128, pl.ds(q0, BQ)]
        cols = []
        for b in range(HQ):
            hh = part + b
            cols.append(jnp.concatenate(
                [qTg[r * DH:(r + 1) * DH, :] if r == hh else zero16 for r in range(HG)],
                axis=0))
        qm = jnp.concatenate(cols, axis=1)
        s_scr[j % 2, 0:nk, :] = jnp.dot(kg, qm, preferred_element_type=F32)

    def attention(blk, first):
        nt = 1 if first else 3
        nk = nt * BQ
        k0 = key_base(blk, nt)
        krow = lax.broadcasted_iota(jnp.int32, (BQ, BQ), 0)
        qcol = lax.broadcasted_iota(jnp.int32, (BQ, BQ), 1)
        diag_ok = jnp.concatenate([krow <= qcol] * HQ, axis=1)
        if not first:
            far = jnp.where(blk >= 2, 0, 2 * BQ)
            far_ok = jnp.concatenate([krow - qcol > far] * HQ, axis=1)

        oT = []

        def softmax_pv(j):
            if first:
                sT = jnp.where(diag_ok, s_scr[j % 2, 0:BQ, :], NEG)
            else:
                sT = jnp.concatenate([
                    jnp.where(far_ok, s_scr[j % 2, 0:BQ, :], NEG),
                    s_scr[j % 2, BQ:2 * BQ, :],
                    jnp.where(diag_ok, s_scr[j % 2, 2 * BQ:3 * BQ, :], NEG)], axis=0)
            m = jnp.max(sT, axis=0, keepdims=True)
            p = jnp.exp2(sT - m)
            l = jnp.sum(p, axis=0, keepdims=True)
            for b in range(HQ):
                h = j * HQ + b
                vTh = vT_scr[h * DH:(h + 1) * DH, pl.ds(k0, nk)]
                oh = lax.dot_general(vTh, p[:, b * BQ:(b + 1) * BQ], (((1,), (0,)), ((), ())),
                                     preferred_element_type=F32)
                oT.append((oh / l[:, b * BQ:(b + 1) * BQ]).astype(BF))

        if first:
            qk(blk, 0, nt)
        for j in range(NQ):
            if j + 1 < NQ:
                qk(blk, j + 1, nt)
            else:
                qk(jnp.minimum(blk + 1, NB - 1), 0, 3)
            if not first and j == EPI_AT:
                epilogue(blk - 1)
            softmax_pv(j)
        oT_scr[blk % 2] = jnp.concatenate(oT, axis=0)

    def out_copy(blk):
        rows = pl.ds(pl.multiple_of(blk * BQ, BQ), BQ)
        return pltpu.make_async_copy(o_buf.at[blk % 2], o_hbm.at[rows], osems.at[blk % 2])

    def epilogue(blk):
        q0 = pl.multiple_of(blk * BQ, BQ)
        aT = jnp.dot(woT_scr[...], oT_scr[blk % 2], preferred_element_type=F32)
        a = aT.T
        xf = x_scr[pl.ds(q0, BQ), :].astype(F32)
        xn = xn_scr[pl.ds(q0, BQ), :].astype(F32)
        grow = lax.broadcasted_iota(jnp.int32, (BQ, D), 0) + q0
        upd = xn * 0.0 + jnp.where(grow == idx_scr[0], y_scr[0:1, :], 0.0)
        o_buf[blk % 2] = (xf + a + (xn + upd)).astype(BF)
        out_copy(blk).start()

    prologue()
    attention(0, True)

    def block_step(blk, carry):
        @pl.when(blk >= 3)
        def _():
            out_copy(blk - 3).wait()

        attention(blk, False)
        return carry

    lax.fori_loop(1, NB, block_step, 0)
    out_copy(NB - 3).wait()
    epilogue(NB - 1)
    out_copy(NB - 2).wait()
    out_copy(NB - 1).wait()


@jax.jit
def pallas_parallel_sum__sliding_block__moe_arch_mod__prompt_kernel(
    A_x, A_wqkv, A_wo, B_x, B_w_r, B_w_gate, B_w_up, B_w_down):
    del B_x
    x = A_x.reshape(S, D)
    wr = B_w_r.reshape(1, D)
    hbm = pl.BlockSpec(memory_space=pl.ANY)
    vm = pltpu.VMEM
    out = pl.pallas_call(
        _kernel,
        in_specs=[hbm] * 7,
        out_specs=hbm,
        out_shape=jax.ShapeDtypeStruct((S, D), A_x.dtype),
        scratch_shapes=[
            vm((S, D), BF), vm((D, 3 * D), BF), vm((D, D), BF), vm((1, D), BF),
            vm((F, D), BF), vm((F, D), BF), vm((F, D), BF),
            vm((S, D), BF),
            vm((D, S), BF),
            vm((S + BQ, D), BF),
            vm((D, S + BQ), BF),
            vm((S, 1), F32),
            vm((8, D), F32),
            pltpu.SMEM((1,), jnp.int32),
            vm((2 * D, D), BF), vm((D, D), BF),
            vm((2, KW, HQ * BQ), F32),
            vm((2, D, BQ), BF),
            vm((2, BQ, D), BF),
            pltpu.SemaphoreType.DMA((_NSEM,)),
            pltpu.SemaphoreType.DMA((2,)),
        ],
        compiler_params=pltpu.CompilerParams(vmem_limit_bytes=100 * 1024 * 1024),
    )(x, A_wqkv, A_wo, wr, B_w_gate.T, B_w_up.T, B_w_down)
    return out.reshape(A_x.shape)
```
